```python
import os as _os
_os.environ.setdefault("JAX_PLATFORMS", "cpu")
import jax
import jax.numpy as jnp

def _softmax(x, axis=-1):
    return jax.nn.softmax(x, axis=axis)
def _gelu(x):
    return jax.nn.gelu(x, approximate=True)
def _silu(x):
    return jax.nn.silu(x)
def _sigmoid(x):
    return jax.nn.sigmoid(x)
def _layernorm(x, axis=-1, eps=1e-5):
    m = jnp.mean(x, axis=axis, keepdims=True)
    v = jnp.var(x, axis=axis, keepdims=True)
    return (x - m) / jnp.sqrt(v + eps)
def _scatter_add(tgt, idx, src, axis=0):
    return tgt.at[idx].add(src)
def _segment_sum(src, seg, n):
    return jax.ops.segment_sum(src, seg, n)
class _Rng:
    def __init__(self, key):
        self._k = key
    def _next(self):
        self._k, sub = jax.random.split(self._k)
        return sub
    def normal(self, shape):
        return jax.random.normal(self._next(), shape, dtype=jnp.bfloat16)
    def randint(self, lo, hi, shape):
        return jax.random.randint(self._next(), shape, lo, hi, dtype=jnp.int32)
    def uniform(self, shape, lo=0.0, hi=1.0):
        return jax.random.uniform(self._next(), shape, jnp.bfloat16, lo, hi)
    def permutation(self, n):
        return jax.random.permutation(self._next(), n)


kernel_name = 'concat_heads__sliding_block_cached__sliding_block_cached__decode'

def setup_inputs():
    _rng = _Rng(jax.random.key(int.from_bytes(__import__("os").urandom(4), "little")))
    _w = (lambda a: (lambda t: t.astype(jnp.bfloat16) if jnp.issubdtype(t.dtype, jnp.floating) else t)(jnp.asarray(a)))
    def _A_setup():
        B, Sq, D = 1, 1, 512
        Hq, Hkv, Sk, Dh = 32, 32, 32768, 128
        assert Hq % Hkv == 0, (Hq, Hkv)
        return {
            "x": _w((lambda *s: _rng.normal(s) * 0.8)(B, Sq, D)),
            "k_cache": _w((lambda *s: _rng.normal(s) * 0.8)(B, Hkv, Sk, Dh)),
            "v_cache": _w((lambda *s: _rng.normal(s) * 0.05)(B, Hkv, Sk, Dh)),
            "wq": _w((lambda *s: _rng.normal(s) * 0.8)(D, Hq * Dh) * (D ** -0.5)),
            "wo": _w((lambda *s: _rng.normal(s) * 0.05)(Hq * Dh, D) * ((Hq * Dh) ** -0.5)),
        }
    _A_in = _A_setup()

    def _B_setup():
        B, Sq, D = 1, 1, 512
        Hq, Hkv, Sk, Dh = 32, 32, 32768, 128
        assert Hq % Hkv == 0, (Hq, Hkv)
        return {
            "x": _w((lambda *s: _rng.normal(s) * 0.8)(B, Sq, D)),
            "k_cache": _w((lambda *s: _rng.normal(s) * 0.8)(B, Hkv, Sk, Dh)),
            "v_cache": _w((lambda *s: _rng.normal(s) * 0.05)(B, Hkv, Sk, Dh)),
            "wq": _w((lambda *s: _rng.normal(s) * 0.8)(D, Hq * Dh) * (D ** -0.5)),
            "wo": _w((lambda *s: _rng.normal(s) * 0.05)(Hq * Dh, D) * ((Hq * Dh) ** -0.5)),
        }
    _B_in = _B_setup()

    return {
        "A_x": _A_in["x"],
        "A_k_cache": _A_in["k_cache"],
        "A_v_cache": _A_in["v_cache"],
        "A_wq": _A_in["wq"],
        "A_wo": _A_in["wo"],
        "B_x": _B_in["x"],
        "B_k_cache": _B_in["k_cache"],
        "B_v_cache": _B_in["v_cache"],
        "B_wq": _B_in["wq"],
        "B_wo": _B_in["wo"],
    }

def reference(A_x, A_k_cache, A_v_cache, A_wq, A_wo, B_x, B_k_cache, B_v_cache, B_wq, B_wo):
    def _A_ref(x, k_cache, v_cache, wq, wo):
        B, Sq, D = x.shape
        Hq, Dh = 32, 128
        Hkv, Sk = k_cache.shape[1], k_cache.shape[2]
        W = min(4096, max(256, Sk // 4))
        rep = Hq // Hkv
        q = (lambda x, *d: x.transpose(*d))((x @ wq).reshape(B, Sq, Hq, Dh), 0, 2, 1, 3)
        k = jnp.repeat(k_cache[:, :, Sk - W:, :], rep, axis=1)
        v = jnp.repeat(v_cache[:, :, Sk - W:, :], rep, axis=1)
        scores = jnp.einsum("bhqd,bhkd->bhqk", q, k) * (Dh ** -0.5)
        p = _softmax(scores, axis=-1)
        o = jnp.einsum("bhqk,bhkd->bhqd", p, v)
        return (lambda x, *d: x.transpose(*d))(o, 0, 2, 1, 3).reshape(B, Sq, Hq * Dh) @ wo

    def _B_ref(x, k_cache, v_cache, wq, wo):
        B, Sq, D = x.shape
        Hq, Dh = 32, 128
        Hkv, Sk = k_cache.shape[1], k_cache.shape[2]
        W = min(4096, max(256, Sk // 4))
        rep = Hq // Hkv
        q = (lambda x, *d: x.transpose(*d))((x @ wq).reshape(B, Sq, Hq, Dh), 0, 2, 1, 3)
        k = jnp.repeat(k_cache[:, :, Sk - W:, :], rep, axis=1)
        v = jnp.repeat(v_cache[:, :, Sk - W:, :], rep, axis=1)
        scores = jnp.einsum("bhqd,bhkd->bhqk", q, k) * (Dh ** -0.5)
        p = _softmax(scores, axis=-1)
        o = jnp.einsum("bhqk,bhkd->bhqd", p, v)
        return (lambda x, *d: x.transpose(*d))(o, 0, 2, 1, 3).reshape(B, Sq, Hq * Dh) @ wo

    a = _A_ref(A_x, A_k_cache, A_v_cache, A_wq, A_wo)
    b = _B_ref(B_x, B_k_cache, B_v_cache, B_wq, B_wo)
    return jnp.concatenate([a, b], axis=-1)
```

```python
import jax
import jax.numpy as jnp
from jax import lax
import jax.experimental.pallas as pl
import jax.experimental.pallas.tpu as pltpu

H, Dh = 32, 128
NS = 2


@jax.jit
def pallas_concat_heads__sliding_block_cached__sliding_block_cached__decode_kernel(
    A_x: jax.Array,
    A_k_cache: jax.Array,
    A_v_cache: jax.Array,
    A_wq: jax.Array,
    A_wo: jax.Array,
    B_x: jax.Array,
    B_k_cache: jax.Array,
    B_v_cache: jax.Array,
    B_wq: jax.Array,
    B_wo: jax.Array,
):
    S = A_k_cache.shape[2]
    D = A_x.shape[2]
    W = min(4096, max(256, S // 4))
    scale = Dh ** -0.5

    def kernel(ax, ak, av, awq, awo, bx, bk, bv, bwq, bwo, o_ref,
               xbuf, kbuf, vbuf, wqbuf, wobuf, acc_ref, xsem, sems):
        def copies(refs, h, slot):
            k, v, wq, wo = refs
            return [
                pltpu.make_async_copy(wq.at[:, pl.ds(pl.multiple_of(h * Dh, Dh), Dh)], wqbuf.at[slot], sems.at[0, slot]),
                pltpu.make_async_copy(k.at[0, h, pl.ds(S - W, W), :], kbuf.at[slot], sems.at[1, slot]),
                pltpu.make_async_copy(v.at[0, h, pl.ds(S - W, W), :], vbuf.at[slot], sems.at[2, slot]),
                pltpu.make_async_copy(wo.at[pl.ds(pl.multiple_of(h * Dh, Dh), Dh), :], wobuf.at[slot], sems.at[3, slot]),
            ]
        A = (ak, av, awq, awo)
        B = (bk, bv, bwq, bwo)
        cx = [pltpu.make_async_copy(ax, xbuf.at[0], xsem.at[0]),
              pltpu.make_async_copy(bx, xbuf.at[1], xsem.at[1])]
        for c in cx:
            c.start()
        L = NS - 1

        def sel(u):
            if u >= 2 * H:
                return None
            return (A, u) if u < H else (B, u - H)

        for u in range(L):
            r, h = sel(u)
            for c in copies(r, h, u % NS):
                c.start()
        for c in cx:
            c.wait()
        acc_ref[...] = jnp.zeros_like(acc_ref)

        def step(u, br, cur, nxt):
            slot = u % NS
            if nxt is not None:
                for c in copies(nxt[0], nxt[1], (u + L) % NS):
                    c.start()
            cs = copies(cur[0], cur[1], slot)
            x = jnp.broadcast_to(xbuf[br, 0], (8, D))
            cs[0].wait()
            q = jnp.dot(x, wqbuf[slot], preferred_element_type=jnp.float32).astype(jnp.bfloat16)
            cs[1].wait()
            s = lax.dot_general(q, kbuf[slot], (((1,), (1,)), ((), ())),
                                preferred_element_type=jnp.float32) * scale
            m = jnp.max(s, axis=-1, keepdims=True)
            p = jnp.exp(s - m)
            l = jnp.sum(p, axis=-1, keepdims=True)
            cs[2].wait()
            o = jnp.dot(p.astype(jnp.bfloat16), vbuf[slot], preferred_element_type=jnp.float32) / l
            cs[3].wait()
            acc_ref[br] += jnp.dot(o.astype(jnp.bfloat16), wobuf[slot], preferred_element_type=jnp.float32)

        lax.fori_loop(0, H - L, lambda u, _: (step(u, 0, (A, u), (A, u + L)), 0)[1], 0)
        for u in range(H - L, H):
            step(u, 0, sel(u), sel(u + L))
        lax.fori_loop(H, 2 * H - L, lambda u, _: (step(u, 1, (B, u - H), (B, u + L - H)), 0)[1], 0)
        for u in range(2 * H - L, 2 * H):
            step(u, 1, sel(u), None)
        o_ref[0, :, 0:D] = acc_ref[0, 0:1, :].astype(o_ref.dtype)
        o_ref[0, :, D:2 * D] = acc_ref[1, 0:1, :].astype(o_ref.dtype)

    return pl.pallas_call(
        kernel,
        out_shape=jax.ShapeDtypeStruct((1, 1, 2 * D), jnp.bfloat16),
        in_specs=[pl.BlockSpec(memory_space=pl.ANY)] * 10,
        out_specs=pl.BlockSpec(memory_space=pltpu.VMEM),
        scratch_shapes=[
            pltpu.VMEM((2, 1, 1, D), jnp.bfloat16),
            pltpu.VMEM((NS, W, Dh), jnp.bfloat16),
            pltpu.VMEM((NS, W, Dh), jnp.bfloat16),
            pltpu.VMEM((NS, D, Dh), jnp.bfloat16),
            pltpu.VMEM((NS, Dh, D), jnp.bfloat16),
            pltpu.VMEM((2, 8, D), jnp.float32),
            pltpu.SemaphoreType.DMA((2,)),
            pltpu.SemaphoreType.DMA((4, NS)),
        ],
        compiler_params=pltpu.CompilerParams(vmem_limit_bytes=64 * 1024 * 1024),
    )(A_x, A_k_cache, A_v_cache, A_wq, A_wo, B_x, B_k_cache, B_v_cache, B_wq, B_wo)
```

```python
import functools
import jax, jax.numpy as jnp
from jax import lax
from jax.experimental import pallas as pl
from jax.experimental.pallas import tpu as pltpu

H, Dh = 32, 128
HG = 4
NU = 2 * HG
R = 512
PR = 32
NEG = -1e30

def make(L1=34, L=59, D0=3, D1=4, nobc=True, compute=True, chain_on=True):
    def f(A_x, A_k, A_v, A_wq, A_wo, B_x, B_k, B_v, B_wq, B_wo):
        S = A_k.shape[2]
        D = A_x.shape[2]
        W = min(4096, max(256, S // 4))
        scale = Dh ** -0.5
        CPG = W // R
        NG = H // HG
        NC = NG * CPG
        assert CPG == 8 and D == 512 and R // NU == 2 * PR
        f32, bf16 = jnp.float32, jnp.bfloat16

        def kernel(ax, ak, av, awq, awo, bx, bk, bv, bwq, bwo, o_ref,
                   xbuf, xb, kbuf, vbuf, wqb, wob, wbig, zref,
                   s_ref, m_ref, l_ref, acc_ref, qacc_ref, q_ref, ocur_ref, out_ref,
                   xsem, sems):
            kv_hbm = ((ak, av), (bk, bv))
            wq_hbm = (awq, bwq)
            wo_hbm = (awo, bwo)
            kv_buf = (kbuf, vbuf)
            st = lambda v: isinstance(v, int)
            def shr(v, n): return v >> n if st(v) else lax.shift_right_logical(v, n)
            def band(v, m): return v & m if st(v) else lax.bitwise_and(v, m)
            def mult(v, m): return v if st(v) else pl.multiple_of(v, m)
            def addz(v, z, hi):
                return v if z is None else jnp.clip(v + z, 0, hi)

            def kv_copy(b, kv, a, row, nrows, z=None):
                c = a - kv
                h0 = addz(shr(c, 3) * HG, z, H - HG)
                src_row = mult(S - W + band(c, CPG - 1) * R + row, PR)
                return pltpu.make_async_copy(
                    kv_hbm[b][kv].at[0, pl.ds(h0, HG), pl.ds(src_row, nrows), :],
                    kv_buf[kv].at[band(c, 3), pl.ds(b * HG, HG), pl.ds(mult(row, PR), nrows), :],
                    sems.at[band(a, 3)])

            def wq_copy(b, g, r32, n32, dst, dr32, sem, z=None):
                r = addz(r32, z, D // 32 - n32)
                return pltpu.make_async_copy(
                    wq_hbm[b].at[pl.ds(mult(r * 32, 32), 32 * n32), pl.ds(mult(g * (HG * Dh), HG * Dh), HG * Dh)],
                    dst.at[b, pl.ds(dr32 * 32, 32 * n32), :], sem)

            def wo_copy(b, r32, n32, dst, dr32, sem, z=None):
                r = addz(r32, z, H * Dh // 32 - n32)
                return pltpu.make_async_copy(
                    wo_hbm[b].at[pl.ds(mult(r * 32, 32), 32 * n32), :],
                    dst.at[b, pl.ds(dr32 * 32, 32 * n32), :], sem)

            def seg_kv(a, u):
                def p0(t, z): return kv_copy(1, t & 1, a, u * 64 + (t >> 1) * PR, PR, z)
                def p1(): return [kv_copy(0, 0, a, u * 64, 64), kv_copy(0, 1, a, u * 64, 64)]
                return p0, p1
            def seg_first(u):
                sem = sems.at[0]
                def p0(t, z):
                    if t & 1 == 0: return kv_copy(1, 0, 0, u * 64 + (t >> 1) * PR, PR, z)
                    return wq_copy(1, 0, 2 * u + (t >> 1), 1, wbig, 2 * u + (t >> 1), sem, z)
                def p1(): return [kv_copy(0, 0, 0, u * 64, 64), wq_copy(0, 0, 2 * u, 2, wbig, 2 * u, sem)]
                return p0, p1
            def seg_wq(a):
                sem = sems.at[band(a, 3)]
                g = shr(a, 3) + 1
                r0 = band(a, 7) * 2
                def p0(t, z): return wq_copy(1, g, r0 + t, 1, wqb, t, sem, z)
                def p1(): return [wq_copy(0, g, r0, 2, wqb, 0, sem), wq_copy(0, g, r0 + 2, 2, wqb, 2, sem)]
                return p0, p1
            def seg_wo(a):
                sem = sems.at[band(a, 3)]
                r0 = shr(a - 8, 1) * 4
                def p0(t, z): return wo_copy(1, r0 + t, 1, wob, t, sem, z)
                def p1(): return [wo_copy(0, r0, 2, wob, 0, sem), wo_copy(0, r0 + 2, 2, wob, 2, sem)]
                return p0, p1
            def seg_last(e):
                if e < 4:
                    def p0(t, z): return kv_copy(1, 1, NC, e * 128 + t * PR, PR, z)
                    def p1(): return [kv_copy(0, 1, NC, e * 128, 64), kv_copy(0, 1, NC, e * 128 + 64, 64)]
                    return p0, p1
                hh = e - 4
                sem = sems.at[(1, 1, 2, 3)[hh]]
                r0 = (H - HG + hh) * 4
                def p0(t, z): return wo_copy(1, r0 + t, 1, wbig, hh * 4 + t, sem, z)
                def p1(): return [wo_copy(0, r0, 2, wbig, hh * 4, sem), wo_copy(0, r0 + 2, 2, wbig, hh * 4 + 2, sem)]
                return p0, p1
            def kvseg_at(a, u):
                if st(a) and st(u):
                    a, u = a + (u >> 3), u & 7
                    if a == 0: return seg_first(u)
                    if a < NC: return seg_kv(a, u)
                    if a == NC: return seg_last(u)
                    return None
                return seg_kv(a + shr(u, 3), band(u, 7))

            def chain(z, n):
                for _ in range(n):
                    z = z * z
                return z

            def run_seg(wseg, s0, s1, work=None):
                if wseg is not None:
                    for t in range(4): wseg[0](t, None).wait()
                    for c in wseg[1](): c.wait()
                z = zref[...][0, 0] if (chain_on and s0 is not None) else None
                if s0 is not None: s0[0](0, None).start(priority=0)
                if s1 is not None:
                    for c in s1[1](): c.start(priority=1)
                res = work() if (work is not None and compute) else None
                if s0 is not None:
                    for t in range(1, 4):
                        if chain_on: z = chain(z, L1 if t == 1 else L)
                        s0[0](t, z).start(priority=0)
                return res

            row8 = lax.broadcasted_iota(jnp.int32, (NU, 128), 0)
            row8w = lax.broadcasted_iota(jnp.int32, (NU, R), 0)

            def qk(q, c, u, s):
                r = lax.dot_general(q, kbuf[band(c, 3), u], (((1,), (1,)), ((), ())), preferred_element_type=f32)
                return jnp.where(row8w == u, r, s)
            def pv(p, c, u, acc):
                r = jnp.dot(p, vbuf[band(c, 3), u], preferred_element_type=f32)
                return jnp.where(row8 == u, acc + r, acc)
            def softmax(first):
                s = s_ref[...]
                mx = jnp.max(s, axis=-1, keepdims=True)
                if first is True:
                    m_new = jnp.broadcast_to(mx, (NU, 128))
                else:
                    m_old = m_ref[...]
                    if first is not False:
                        m_old = jnp.where(first, NEG, m_old)
                    m_new = jnp.maximum(m_old, mx)
                ps = [jnp.exp((s[:, t * 128:(t + 1) * 128] - m_new) * scale) for t in range(R // 128)]
                ls = (ps[0] + ps[1]) + (ps[2] + ps[3])
                p = jnp.concatenate(ps, axis=1)
                if first is True:
                    l_new = ls
                    acc = jnp.zeros((NU, 128), f32)
                else:
                    alpha = jnp.exp((m_old - m_new) * scale)
                    l_s = l_ref[...] * alpha
                    acc = acc_ref[...] * alpha
                    if first is not False:
                        l_s = jnp.where(first, 0.0, l_s)
                        acc = jnp.where(first, 0.0, acc)
                    l_new = l_s + ls
                m_ref[...] = m_new
                l_ref[...] = l_new
                return p.astype(bf16), acc
            def finalize():
                l = jnp.sum(l_ref[...], axis=-1, keepdims=True)
                return (acc_ref[...] / l).astype(bf16)
            def qproj(wref, r0, blk):
                acc = jnp.zeros((NU, 128), f32)
                for b in range(2):
                    r = jnp.dot(xb[b, blk], wref[b, r0:r0 + 128, :], preferred_element_type=f32)
                    for hh in range(HG):
                        acc = jnp.where(row8 == b * HG + hh, r[:, hh * 128:(hh + 1) * 128], acc)
                return acc
            def outproj(o, wref, r0, hh):
                out = out_ref[...]
                for b in range(2):
                    r = jnp.dot(o, wref[b, r0:r0 + 128, :], preferred_element_type=f32)
                    out = jnp.where(row8w == b * HG + hh, out + r, out)
                out_ref[...] = out

            def wwork_odd(a, do_sm=True):
                def fn():
                    j1 = band(a, 7) == 1
                    res = softmax(False) if do_sm else None
                    qa = qacc_ref[...]
                    q_ref[...] = jnp.where(j1, qa.astype(bf16), q_ref[...])
                    qacc_ref[...] = jnp.where(j1, 0.0, qa) + qproj(wqb, 0, shr(band(a, 7), 1))
                    return res
                return fn
            def wwork_even(a, do_out):
                def fn():
                    first = band(a - 2, 7) == 0
                    if do_out:
                        o = jnp.where(first, finalize(), ocur_ref[...])
                        ocur_ref[...] = o
                        outproj(o, wob, 0, band(shr(a - 2, 1), 3))
                    return softmax(first)
                return fn

            def units_loop(a, pa, lo=0, hi=NU, carry=None):
                q = q_ref[...]
                def body(u, carry):
                    def work():
                        s, acc = carry
                        if pa is not None:
                            acc = pv(pa[0], a - 2, u, acc)
                        return qk(q, a - 1, u, s), acc
                    res = run_seg(kvseg_at(a, u), kvseg_at(a, u + D0), kvseg_at(a, u + D1), work)
                    return res if res is not None else carry
                if carry is None:
                    carry = (jnp.zeros((NU, R), f32), pa[1] if pa is not None else jnp.zeros((NU, 128), f32))
                return lax.fori_loop(lo, hi, body, carry), body

            def phase(a, wseg, wwork):
                pa = run_seg(wseg, wseg, wseg, wwork)
                if not compute: pa = (None, jnp.zeros((NU, 128), f32))
                (s, acc), _ = units_loop(a, pa)
                s_ref[...] = s
                acc_ref[...] = acc

            zref[...] = jnp.zeros(zref.shape, jnp.int32)
            cx = [pltpu.make_async_copy(ax, xbuf.at[0], xsem.at[0]), pltpu.make_async_copy(bx, xbuf.at[1], xsem.at[1])]
            for u in range(D1):
                for c in kvseg_at(0, u)[1](): c.start(priority=1)
            for c in cx: c.start()
            for u in range(D0):
                for t in range(4): kvseg_at(0, u)[0](t, None).start(priority=0)
            out_ref[...] = jnp.zeros(out_ref.shape, f32)
            ocur_ref[...] = jnp.zeros(ocur_ref.shape, bf16)
            q_ref[...] = jnp.zeros(q_ref.shape, bf16)
            for c in cx: c.wait()
            for b in range(2):
                xv = jnp.broadcast_to(xbuf[b, 0], (NU, D))
                for t in range(D // 128):
                    xb[b, t] = xv[:, t * 128:(t + 1) * 128]
            run_seg(seg_wq(0), seg_wq(0), seg_wq(0))
            for u in range(NU):
                run_seg(kvseg_at(0, u), kvseg_at(0, u + D0), kvseg_at(0, u + D1))
            if compute:
                q0 = qproj(wbig, 0, 0)
                for t in range(1, 4):
                    q0 = q0 + qproj(wbig, t * 128, t)
                qacc_ref[...] = q0
                wwork_odd(1, do_sm=False)()
            (s, acc), _ = units_loop(jnp.int32(1), None)
            s_ref[...] = s
            m_ref[...] = jnp.zeros(m_ref.shape, f32)
            l_ref[...] = jnp.zeros(l_ref.shape, f32)
            acc_ref[...] = acc
            phase(jnp.int32(2), seg_wq(2), wwork_even(2, False))

            def pair(has_wo, has_wq, i, _):
                a = 2 * i + 1
                phase(a, seg_wo(a) if has_wo else None, wwork_odd(a))
                phase(a + 1, seg_wq(a + 1) if has_wq else None, wwork_even(a + 1, has_wo))
                return 0
            lax.fori_loop(1, 4, functools.partial(pair, False, True), 0)
            lax.fori_loop(4, 27, functools.partial(pair, True, True), 0)
            lax.fori_loop(27, 31, functools.partial(pair, True, False), 0)

            a = NC - 1
            pa = run_seg(seg_wo(a), seg_wo(a), seg_wo(a), lambda: softmax(False))
            if not compute: pa = (None, jnp.zeros((NU, 128), f32))
            npeel = max(D0, D1)
            carry, _ = units_loop(jnp.int32(a), pa, 0, NU - npeel)
            q = q_ref[...]
            for u in range(NU - npeel, NU):
                def work(u=u, carry=carry):
                    s, acc = carry
                    return qk(q, a - 1, u, s), pv(pa[0], a - 2, u, acc)
                r = run_seg(kvseg_at(a, u), kvseg_at(a, u + D0), kvseg_at(a, u + D1), work)
                carry = r if r is not None else carry
            s_ref[...] = carry[0]
            acc_ref[...] = carry[1]

            a = NC
            E = {}
            def w0():
                outproj(ocur_ref[...], wob, 0, 3)
                E["p"], E["acc"] = softmax(False)
                s = jnp.zeros((NU, R), f32)
                for u in range(0, 3): s = qk(q, a - 1, u, s)
                E["s"] = s
            def w1():
                for u in range(3, 6): E["s"] = qk(q, a - 1, u, E["s"])
                for u in range(0, 3): E["acc"] = pv(E["p"], a - 2, u, E["acc"])
            def w2():
                for u in range(6, 8): E["s"] = qk(q, a - 1, u, E["s"])
                for u in range(3, 8): E["acc"] = pv(E["p"], a - 2, u, E["acc"])
                s_ref[...] = E["s"]
                acc_ref[...] = E["acc"]
            def w3():
                E["p"], E["acc"] = softmax(False)
            def w4():
                for u in range(8): E["acc"] = pv(E["p"], a - 1, u, E["acc"])
                acc_ref[...] = E["acc"]
            def w5():
                E["o"] = finalize()
            def w6():
                outproj(E["o"], wbig, 0, 0)
                outproj(E["o"], wbig, 128, 1)
            def w7():
                outproj(E["o"], wbig, 256, 2)
            works = [w0, w1, w2, w3, w4, w5, w6, w7]
            if compute: w0()
            for e in range(8):
                nxt = works[e + 1] if e + 1 < 8 else (lambda: outproj(E["o"], wbig, 384, 3))
                run_seg(kvseg_at(a, e), kvseg_at(a, e + D0), kvseg_at(a, e + D1), nxt)
            out = out_ref[...]
            for b in range(2):
                o_ref[0, :, b * D:(b + 1) * D] = jnp.sum(out[b * HG:(b + 1) * HG], axis=0, keepdims=True).astype(o_ref.dtype)

        return pl.pallas_call(
            kernel,
            out_shape=jax.ShapeDtypeStruct((1, 1, 2 * D), jnp.bfloat16),
            in_specs=[pl.BlockSpec(memory_space=pl.ANY)] * 10,
            out_specs=pl.BlockSpec(memory_space=pltpu.VMEM),
            scratch_shapes=[
                pltpu.VMEM((2, 1, 1, D), bf16),
                pltpu.VMEM((2, D // 128, NU, 128), bf16),
                pltpu.VMEM((4, NU, R, Dh), bf16),
                pltpu.VMEM((4, NU, R, Dh), bf16),
                pltpu.VMEM((2, 128, HG * Dh), bf16),
                pltpu.VMEM((2, 128, D), bf16),
                pltpu.VMEM((2, 512, 512), bf16),
                pltpu.VMEM((8, 128), jnp.int32),
                pltpu.VMEM((NU, R), f32),
                pltpu.VMEM((NU, 128), f32),
                pltpu.VMEM((NU, 128), f32),
                pltpu.VMEM((NU, 128), f32),
                pltpu.VMEM((NU, 128), f32),
                pltpu.VMEM((NU, 128), bf16),
                pltpu.VMEM((NU, 128), bf16),
                pltpu.VMEM((NU, D), f32),
                pltpu.SemaphoreType.DMA((2,)),
                pltpu.SemaphoreType.DMA((4,)),
            ],
            compiler_params=pltpu.CompilerParams(vmem_limit_bytes=64 * 1024 * 1024, disable_bounds_checks=nobc),
        )(A_x, A_k, A_v, A_wq, A_wo, B_x, B_k, B_v, B_wq, B_wo)
    return f


_impl = make(D1=5, nobc=False)


@jax.jit
def pallas_concat_heads__sliding_block_cached__sliding_block_cached__decode_kernel(
    A_x: jax.Array,
    A_k_cache: jax.Array,
    A_v_cache: jax.Array,
    A_wq: jax.Array,
    A_wo: jax.Array,
    B_x: jax.Array,
    B_k_cache: jax.Array,
    B_v_cache: jax.Array,
    B_wq: jax.Array,
    B_wo: jax.Array,
):
    return _impl(A_x, A_k_cache, A_v_cache, A_wq, A_wo, B_x, B_k_cache, B_v_cache, B_wq, B_wo)
```

```python
import functools
import jax, jax.numpy as jnp
from jax import lax
from jax.experimental import pallas as pl
from jax.experimental.pallas import tpu as pltpu

H, Dh = 32, 128
HG = 4
NU = 2 * HG
R = 512
PR = 32
NEG = -1e30

def make(L1=34, L=59, D0=3, D1=5, nobc=True, compute=True, GX=0, L0=55):
    def f(A_x, A_k, A_v, A_wq, A_wo, B_x, B_k, B_v, B_wq, B_wo):
        S = A_k.shape[2]
        D = A_x.shape[2]
        W = min(4096, max(256, S // 4))
        scale = Dh ** -0.5
        CPG = W // R
        NG = H // HG
        NC = NG * CPG
        NB = D // 128
        GW = HG * Dh
        assert CPG == 8 and D == 512 and R // NU == 2 * PR
        f32, bf16 = jnp.float32, jnp.bfloat16

        def kernel(ax, ak, av, awq, awo, bx, bk, bv, bwq, bwo, o_ref,
                   xbuf, xb, kbuf, vbuf, wqr, wor, zref,
                   s_ref, m_ref, l_ref, acc_ref, q_ref, ocur_ref, out_ref,
                   xsem, sems):
            kv_hbm = ((ak, av), (bk, bv))
            wq_hbm = (awq, bwq)
            wo_hbm = (awo, bwo)
            kv_buf = (kbuf, vbuf)
            st = lambda v: isinstance(v, int)
            def shr(v, n): return v >> n if st(v) else lax.shift_right_logical(v, n)
            def band(v, m): return v & m if st(v) else lax.bitwise_and(v, m)
            def mult(v, m): return v if st(v) else pl.multiple_of(v, m)
            def gmap(b, g):
                if b == 0 or GX == 0: return g
                return g ^ GX if st(g) else lax.bitwise_xor(g, GX)
            def addz(v, z, hi):
                return v if z is None else jnp.clip(v + z, 0, hi)

            def kv_copy(b, kv, a, row, z=None):
                c = a - kv
                h0 = addz(gmap(b, shr(c, 3)) * HG, z, H - HG)
                src_row = mult(S - W + band(c, CPG - 1) * R + row, PR)
                return pltpu.make_async_copy(
                    kv_hbm[b][kv].at[0, pl.ds(h0, HG), pl.ds(src_row, PR), :],
                    kv_buf[kv].at[band(c, 3), pl.ds(b * HG, HG), pl.ds(mult(row, PR), PR), :],
                    sems.at[band(a, 3)])
            def wq_copy(b, g, r, sem, z=None):
                rs = addz(r, z, 15)
                return pltpu.make_async_copy(
                    wq_hbm[b].at[:, pl.ds(mult(rs * 8, 8), 8), pl.ds(gmap(b, g) * GW, GW)],
                    wqr.at[b, g, :, pl.ds(mult(r * 8, 8), 8), :], sem)
            def wo_copy(b, g, r, sem, z=None):
                rs = addz(r, z, 15)
                return pltpu.make_async_copy(
                    wo_hbm[b].at[pl.ds(mult(gmap(b, g) * GW + rs * PR, PR), PR), :],
                    wor.at[b, pl.ds(mult(g * GW + r * PR, PR), PR), :], sem)

            def seg_kv(a, u):
                return lambda b, t, z=None: kv_copy(b, t & 1, a, u * 64 + (t >> 1) * PR, z)
            def seg_first(u):
                def pc(b, t, z=None):
                    if t & 1 == 0: return kv_copy(b, 0, 0, u * 64 + (t >> 1) * PR, z)
                    return wq_copy(b, NG - 1, 2 * u + (t >> 1), sems.at[0], z)
                return pc
            def seg_last(e):
                if e < 4:
                    return lambda b, t, z=None: kv_copy(b, 1, NC, e * 128 + t * PR, z)
                hh = e - 4
                sem = sems.at[(1, 1, 2, 3)[hh]]
                return lambda b, t, z=None: wo_copy(b, NG - 1, hh * 4 + t, sem, z)
            def seg_at(a, u):
                if st(a) and st(u):
                    a, u = a + (u >> 3), u & 7
                    if a == 0: return seg_first(u)
                    if a < NC: return seg_kv(a, u)
                    if a == NC: return seg_last(u)
                    return None
                return seg_kv(a + shr(u, 3), band(u, 7))

            def chain(z, n):
                for _ in range(n):
                    z = z * z
                return z

            def run_seg(a, u, work=None):
                wseg, s0, s1 = seg_at(a, u), seg_at(a, u + D0), seg_at(a, u + D1)
                for b in range(2):
                    for t in range(4): wseg(b, t).wait()
                z = zref[...][0, 0] if s0 is not None else None
                if s0 is not None: s0(1, 0).start(priority=0)
                if s1 is not None:
                    for t in range(4): s1(0, t).start(priority=1)
                res = work() if (work is not None and compute) else None
                if s0 is not None:
                    for t in range(1, 4):
                        z = chain(z, L1 if t == 1 else L)
                        s0(1, t, z).start(priority=0)
                return res

            row8 = lax.broadcasted_iota(jnp.int32, (NU, 128), 0)
            row8w = lax.broadcasted_iota(jnp.int32, (NU, R), 0)

            def qk(q, c, u, s):
                r = lax.dot_general(q, kbuf[band(c, 3), u], (((1,), (1,)), ((), ())), preferred_element_type=f32)
                return r if s is None else jnp.where(row8w == u, r, s)
            def pv(p, c, u, acc):
                r = jnp.dot(p, vbuf[band(c, 3), u], preferred_element_type=f32)
                return jnp.where(row8 == u, acc + r, acc)
            def softmax(first):
                s = s_ref[...]
                mx = jnp.max(s, axis=-1, keepdims=True)
                m_old = m_ref[...]
                if first is not False:
                    m_old = jnp.where(first, NEG, m_old)
                m_new = jnp.maximum(m_old, mx)
                ps = [jnp.exp((s[:, t * 128:(t + 1) * 128] - m_new) * scale) for t in range(R // 128)]
                ls = (ps[0] + ps[1]) + (ps[2] + ps[3])
                p = jnp.concatenate(ps, axis=1)
                alpha = jnp.exp((m_old - m_new) * scale)
                l_s = l_ref[...] * alpha
                acc = acc_ref[...] * alpha
                if first is not False:
                    l_s = jnp.where(first, 0.0, l_s)
                    acc = jnp.where(first, 0.0, acc)
                m_ref[...] = m_new
                l_ref[...] = l_s + ls
                return p.astype(bf16), acc
            def finalize():
                l = jnp.sum(l_ref[...], axis=-1, keepdims=True)
                return (acc_ref[...] / l).astype(bf16)
            def qproj(g):
                q = jnp.zeros((NU, 128), f32)
                for b in range(2):
                    r = jnp.dot(xb[b, 0], wqr[b, g, 0], preferred_element_type=f32)
                    for t in range(1, NB):
                        r = r + jnp.dot(xb[b, t], wqr[b, g, t], preferred_element_type=f32)
                    for hh in range(HG):
                        q = jnp.where(row8 == b * HG + hh, r[:, hh * 128:(hh + 1) * 128], q)
                q_ref[g] = q.astype(bf16)
            def outproj(o, g, v, valid=None):
                r0 = mult(g * GW + band(v, HG - 1) * Dh, Dh)
                r = jnp.dot(o, wor[shr(v, 2), pl.ds(r0, Dh), :], preferred_element_type=f32)
                out = out_ref[...]
                sel = row8w == (v if valid is None else jnp.where(valid, v, -1))
                out_ref[...] = jnp.where(sel, out + r, out)

            def head_work(a):
                q = q_ref[shr(a - 1, 3)]
                v = band(a - 2, 7)
                first = v == 0
                o = jnp.where(first, finalize(), ocur_ref[...])
                ocur_ref[...] = o
                g1 = shr(a - 2, 3)
                outproj(o, jnp.maximum(g1 - 1, 0), v, g1 >= 1)
                p, acc = softmax(first)
                return q, p, qk(q, a - 1, 0, None), pv(p, a - 2, 0, acc)

            def phase(a, hi=NU):
                r = run_seg(a, 0, lambda: head_work(a))
                if r is None: r = (None, None, jnp.zeros((NU, R), f32), jnp.zeros((NU, 128), f32))
                q, p, s, acc = r
                def body(u, carry, a=a):
                    res = run_seg(a, u, lambda: (qk(q, a - 1, u, carry[0]), pv(p, a - 2, u, carry[1])))
                    return res if res is not None else carry
                carry = lax.fori_loop(1, hi, body, (s, acc))
                for u in range(hi, NU):
                    carry = body(u, carry, NC - 1)
                s_ref[...] = carry[0]
                acc_ref[...] = carry[1]

            NX = 2 * (NG - 1)
            d0, d1 = 4 * D0 - 3, 4 * D1
            xs = sems.at[3]
            def xpiece(b, r, k, z=None):
                r, k = r + k // NX, k % NX
                if st(r) and r >= 16:
                    n = (r - 16) * NX + k
                    return seg_at(0, n // 4)(b, n % 4, z)
                return (wq_copy if k % 2 == 0 else wo_copy)(b, k // 2, r, xs, z)
            zref[...] = jnp.zeros(zref.shape, jnp.int32)
            cx = [pltpu.make_async_copy(ax, xbuf.at[0], xsem.at[0]), pltpu.make_async_copy(bx, xbuf.at[1], xsem.at[1])]
            xpiece(0, 0, 0).start(priority=1)
            xpiece(1, 0, 0).start(priority=0)
            for k in range(1, d1): xpiece(0, 0, k).start(priority=1)
            for c in cx: c.start(priority=1)
            z = zref[...][0, 0] if L0 else None
            for k in range(1, d0):
                if L0 and k > 1: z = chain(z, L0)
                xpiece(1, 0, k, z).start(priority=0)
            out_ref[...] = jnp.zeros(out_ref.shape, f32)
            ocur_ref[...] = jnp.zeros(ocur_ref.shape, bf16)
            m_ref[...] = jnp.zeros(m_ref.shape, f32)
            l_ref[...] = jnp.ones(l_ref.shape, f32)
            acc_ref[...] = jnp.zeros(acc_ref.shape, f32)
            def xstep(r, _):
                for k in range(NX):
                    xpiece(0, r, k).wait(); xpiece(1, r, k).wait()
                    xpiece(1, r, k + d0).start(priority=0)
                    xpiece(0, r, k + d1).start(priority=1)
                return 0
            npeel = -(-max(d0, d1) // NX)
            lax.fori_loop(0, 16 - npeel, xstep, 0)
            for r in range(16 - npeel, 16): xstep(r, 0)
            z = zref[...][0, 0]
            for c in cx: c.wait()
            for b in range(2):
                xv = jnp.broadcast_to(xbuf[b, 0], (NU, D))
                for t in range(NB):
                    xb[b, t] = xv[:, t * 128:(t + 1) * 128]
            for t in range(1, 4):
                z = chain(z, L1 if t == 1 else L)
                xpiece(1, 16, d0 - 1 + t, z).start(priority=0)
            for u in range(NU):
                run_seg(0, u, functools.partial(qproj, u))
            a1 = jnp.int32(1)
            q = q_ref[0]
            s = run_seg(1, 0, lambda: qk(q, 0, 0, None))
            if s is None: s = jnp.zeros((NU, R), f32)
            def body1(u, s):
                res = run_seg(a1, u, lambda: qk(q, 0, u, s))
                return res if res is not None else s
            s_ref[...] = lax.fori_loop(1, NU, body1, s)

            lax.fori_loop(2, NC - 1, lambda a, _: (phase(a), 0)[1], 0)
            phase(jnp.int32(NC - 1), hi=NU - max(D0, D1))

            a = NC
            E = {}
            q = q_ref[NG - 1]
            def w0():
                E["p"], E["acc"] = softmax(False)
                s = qk(q, a - 1, 0, None)
                for u in range(1, 3): s = qk(q, a - 1, u, s)
                E["s"] = s
            def w1():
                for u in range(3, 6): E["s"] = qk(q, a - 1, u, E["s"])
                for u in range(0, 3): E["acc"] = pv(E["p"], a - 2, u, E["acc"])
            def w2():
                for u in range(6, 8): E["s"] = qk(q, a - 1, u, E["s"])
                for u in range(3, 8): E["acc"] = pv(E["p"], a - 2, u, E["acc"])
                s_ref[...] = E["s"]
                acc_ref[...] = E["acc"]
            def w3():
                E["p"], E["acc"] = softmax(False)
                for v in (6, 7): outproj(ocur_ref[...], NG - 2, v)
            def w4():
                for u in range(8): E["acc"] = pv(E["p"], a - 1, u, E["acc"])
                acc_ref[...] = E["acc"]
            def w5():
                E["o"] = finalize()
            def wo_(hhs):
                def fn():
                    for hh in hhs:
                        for b in range(2): outproj(E["o"], NG - 1, b * HG + hh)
                return fn
            works = [w0, w1, w2, w3, w4, w5, wo_((0, 1)), wo_((2,)), wo_((3,))]
            if compute: w0()
            for e in range(8):
                run_seg(a, e, works[e + 1])
            out = out_ref[...]
            for b in range(2):
                o_ref[0, :, b * D:(b + 1) * D] = jnp.sum(out[b * HG:(b + 1) * HG], axis=0, keepdims=True).astype(o_ref.dtype)

        return pl.pallas_call(
            kernel,
            out_shape=jax.ShapeDtypeStruct((1, 1, 2 * D), jnp.bfloat16),
            in_specs=[pl.BlockSpec(memory_space=pl.ANY)] * 10,
            out_specs=pl.BlockSpec(memory_space=pltpu.VMEM),
            scratch_shapes=[
                pltpu.VMEM((2, 1, 1, D), bf16),
                pltpu.VMEM((2, NB, NU, 128), bf16),
                pltpu.VMEM((4, NU, R, Dh), bf16),
                pltpu.VMEM((4, NU, R, Dh), bf16),
                pltpu.VMEM((2, NG, NB, 128, GW), bf16),
                pltpu.VMEM((2, H * Dh, D), bf16),
                pltpu.VMEM((8, 128), jnp.int32),
                pltpu.VMEM((NU, R), f32),
                pltpu.VMEM((NU, 128), f32),
                pltpu.VMEM((NU, 128), f32),
                pltpu.VMEM((NU, 128), f32),
                pltpu.VMEM((NG, NU, 128), bf16),
                pltpu.VMEM((NU, 128), bf16),
                pltpu.VMEM((NU, D), f32),
                pltpu.SemaphoreType.DMA((2,)),
                pltpu.SemaphoreType.DMA((4,)),
            ],
            compiler_params=pltpu.CompilerParams(vmem_limit_bytes=64 * 1024 * 1024, disable_bounds_checks=nobc),
        )(A_x, A_k, A_v, A_wq.reshape(NB, 128, H * Dh), A_wo, B_x, B_k, B_v, B_wq.reshape(NB, 128, H * Dh), B_wo)
    return f


_impl = make(GX=4)


@jax.jit
def pallas_concat_heads__sliding_block_cached__sliding_block_cached__decode_kernel(
    A_x: jax.Array,
    A_k_cache: jax.Array,
    A_v_cache: jax.Array,
    A_wq: jax.Array,
    A_wo: jax.Array,
    B_x: jax.Array,
    B_k_cache: jax.Array,
    B_v_cache: jax.Array,
    B_wq: jax.Array,
    B_wo: jax.Array,
):
    return _impl(A_x, A_k_cache, A_v_cache, A_wq, A_wo, B_x, B_k_cache, B_v_cache, B_wq, B_wo)
```

```python
import jax
import jax.numpy as jnp
from jax import lax
import jax.experimental.pallas as pl
import jax.experimental.pallas.tpu as pltpu

H, DH = 32, 128
HG = 4
NU = 2 * HG
R = 512
KR = 16
WR = 32
AHEAD = (20, 12)
SPIN0, SPIN1, SPIN = 50, 30, 54


@jax.jit
def pallas_concat_heads__sliding_block_cached__sliding_block_cached__decode_kernel(
    A_x: jax.Array,
    A_k_cache: jax.Array,
    A_v_cache: jax.Array,
    A_wq: jax.Array,
    A_wo: jax.Array,
    B_x: jax.Array,
    B_k_cache: jax.Array,
    B_v_cache: jax.Array,
    B_wq: jax.Array,
    B_wo: jax.Array,
):
    S = A_k_cache.shape[2]
    D = A_x.shape[2]
    W = min(4096, max(256, S // 4))
    scale = DH ** -0.5
    CPG = W // R
    NG = H // HG
    NC = NG * CPG
    NB = D // 128
    GW = HG * DH
    NRS = GW // WR
    assert A_x.shape == (1, 1, 512) and A_k_cache.shape == (1, H, S, DH)
    assert CPG == NU and NG == NU and R == 4 * KR * NU and NRS * 8 == 128
    f32, bf16 = jnp.float32, jnp.bfloat16

    def kernel(ax, ak, av, awq, awo, bx, bk, bv, bwq, bwo, o_ref,
               xbuf, xb, kbuf, vbuf, wqr, wor, zref,
               s_ref, m_ref, l_ref, acc_ref, q_ref, ocur_ref, out_ref, sems):
        kv_hbm = ((ak, av), (bk, bv))
        wq_hbm = (awq, bwq)
        wo_hbm = (awo, bwo)
        kv_buf = (kbuf, vbuf)

        def static(v):
            return isinstance(v, int)

        def shr(v, n):
            return v >> n if static(v) else lax.shift_right_logical(v, n)

        def band(v, m):
            return v & m if static(v) else lax.bitwise_and(v, m)

        def mult(v, m):
            return v if static(v) else pl.multiple_of(v, m)

        def gmap(b, g):
            return g ^ b if static(g) else lax.bitwise_xor(g, b)

        def paced(v, z, hi):
            return v if z is None else jnp.clip(v + z, 0, hi)

        def spin(z, n):
            for _ in range(n):
                z = z * z
            return z

        def kv_piece(b, c, n, z=None):
            h0 = paced(gmap(b, shr(c, 3)) * HG, z, H - HG)
            row = mult(n * KR, KR)
            src_row = mult(S - W + band(c, CPG - 1) * R + row, KR)
            return [pltpu.make_async_copy(
                kv_hbm[b][kv].at[0, pl.ds(h0, HG), pl.ds(src_row, KR), :],
                kv_buf[kv].at[band(c, 3), pl.ds(b * HG, HG), pl.ds(row, KR), :],
                sems.at[band(c, 3)]) for kv in range(2)]

        def wq_piece(b, g, r, sem, z=None):
            return [pltpu.make_async_copy(
                wq_hbm[b].at[:, pl.ds(mult(paced(r, z, NRS - 1) * 8, 8), 8), pl.ds(g * GW, GW)],
                wqr.at[b, gmap(b, g), :, pl.ds(mult(r * 8, 8), 8), :], sem)]

        def wo_piece(b, g, r, sem, z=None):
            return [pltpu.make_async_copy(
                wo_hbm[b].at[pl.ds(mult(gmap(b, g) * GW + paced(r, z, NRS - 1) * WR, WR), WR), :],
                wor.at[b, pl.ds(mult(g * GW + r * WR, WR), WR), :], sem)]

        def piece(b, a, u, t, z=None):
            u, t = u + t // 4, t % 4
            a, u = a + shr(u, 3), band(u, 7)
            if not static(a) or a < NC:
                return kv_piece(b, a, 4 * u + t, z)
            if a > NC:
                return []
            r = 4 * (u & 3) + t if u >= 6 else 4 * ((u & 2) + (t & 1)) + 2 * (u & 1) + (t >> 1)
            return wo_piece(b, NG - 2 + (u >> 2), r, sems.at[(0, 0, 1, 1, 2, 2, 3, 0)[u]], z)

        def start(b, copies):
            for c in copies:
                c.start(priority=1 - b)

        def wait(copies):
            for c in copies:
                c.wait()

        def segment(a, u, work):
            for b in range(2):
                for t in range(4):
                    wait(piece(b, a, u, t))
            more = not (static(a) and static(u) and 32 * a + 4 * u + 1 + AHEAD[1] >= 32 * (NC + 1))
            z = zref[...][0, 0] if more else None
            start(1, piece(1, a, u, AHEAD[1]))
            start(0, piece(0, a, u, AHEAD[0]))
            res = work()
            for t in range(1, 4):
                if more:
                    z = spin(z, SPIN1 if t == 1 else SPIN)
                    start(1, piece(1, a, u, t + AHEAD[1], z))
                start(0, piece(0, a, u, t + AHEAD[0]))
            return res

        row_n = lax.broadcasted_iota(jnp.int32, (NU, DH), 0)
        row_w = lax.broadcasted_iota(jnp.int32, (NU, R), 0)

        def qk(q, c, u, s):
            r = lax.dot_general(q, kbuf[band(c, 3), u], (((1,), (1,)), ((), ())),
                                preferred_element_type=f32)
            return r if s is None else jnp.where(row_w == u, r, s)

        def pv(p, c, u, acc):
            r = jnp.dot(p, vbuf[band(c, 3), u], preferred_element_type=f32)
            return jnp.where(row_n == u, acc + r, acc)

        def softmax(first):
            s = s_ref[...]
            mx = jnp.broadcast_to(jnp.max(s, axis=-1, keepdims=True), (NU, DH))
            m_old = m_ref[...]
            m_new = jnp.maximum(m_old, mx)
            if first is not None:
                m_new = jnp.where(first, mx, m_new)
            ps = [jnp.exp((s[:, t * 128:(t + 1) * 128] - m_new) * scale) for t in range(R // 128)]
            alpha = jnp.exp((m_old - m_new) * scale)
            l_old = l_ref[...] * alpha
            acc = acc_ref[...] * alpha
            if first is not None:
                l_old = jnp.where(first, 0.0, l_old)
                acc = jnp.where(first, 0.0, acc)
            m_ref[...] = m_new
            l_ref[...] = l_old + ((ps[0] + ps[1]) + (ps[2] + ps[3]))
            return jnp.concatenate(ps, axis=1).astype(bf16), acc

        def normalized():
            return acc_ref[...] / jnp.sum(l_ref[...], axis=-1, keepdims=True)

        def qproj(g):
            q = jnp.zeros((NU, DH), f32)
            for b in range(2):
                r = jnp.dot(xb[b, 0], wqr[b, g, 0], preferred_element_type=f32)
                for t in range(1, NB):
                    r = r + jnp.dot(xb[b, t], wqr[b, g, t], preferred_element_type=f32)
                for hh in range(HG):
                    q = jnp.where(row_n == b * HG + hh, r[:, hh * DH:(hh + 1) * DH], q)
            q_ref[g] = q.astype(bf16)

        def outproj(o, g, v, valid=None):
            r0 = mult(g * GW + band(v, HG - 1) * DH, DH)
            r = jnp.dot(o, wor[shr(v, 2), pl.ds(r0, DH), :], preferred_element_type=f32)
            out = out_ref[...]
            sel = row_w == (v if valid is None else jnp.where(valid, v, -1))
            out_ref[...] = jnp.where(sel, out + r, out)

        def head_work(a):
            q = q_ref[shr(a - 1, 3)]
            v = band(a - 2, 7)
            first = v == 0
            o = jnp.where(first, normalized().astype(bf16), ocur_ref[...])
            ocur_ref[...] = o
            g1 = shr(a - 2, 3)
            outproj(o, jnp.clip(g1 - 1, 0, NG - 3), v, jnp.logical_and(g1 >= 1, g1 <= NG - 2))
            p, acc = softmax(first)
            return q, p, qk(q, a - 1, 0, None), pv(p, a - 2, 0, acc)

        def phase(a, hi=NU):
            q, p, s, acc = segment(a, 0, lambda: head_work(a))

            def body(u, carry):
                return segment(a, u, lambda: (qk(q, a - 1, u, carry[0]), pv(p, a - 2, u, carry[1])))

            carry = lax.fori_loop(1, hi, body, (s, acc))
            for u in range(hi, NU):
                carry = body(u, carry)
            s_ref[...] = carry[0]
            acc_ref[...] = carry[1]

        order = []
        for g in range(NG):
            order.append((wq_piece, g))
            if g % 4 != 3:
                order.append((wo_piece, g - g // 4))
        NX = len(order)
        ahead = [n - 3 for n in AHEAD]
        xsem = sems.at[3]

        def xpiece(b, r, k, z=None):
            r, k = r + k // NX, k % NX
            if static(r) and r >= NRS:
                return piece(b, 0, 0, (r - NRS) * NX + k, z)
            return order[k][0](b, order[k][1], r, xsem, z)

        cx = [pltpu.make_async_copy(ax, xbuf.at[0], xsem), pltpu.make_async_copy(bx, xbuf.at[1], xsem)]
        start(0, xpiece(0, 0, 0))
        start(1, xpiece(1, 0, 0))
        zref[...] = jnp.zeros(zref.shape, jnp.int32)
        for k in range(1, ahead[0]):
            start(0, xpiece(0, 0, k))
        start(0, cx)
        z = zref[...][0, 0]
        for k in range(1, ahead[1]):
            if k > 1:
                z = spin(z, SPIN0)
            start(1, xpiece(1, 0, k, z))
        out_ref[...] = jnp.zeros(out_ref.shape, f32)
        ocur_ref[...] = jnp.zeros(ocur_ref.shape, bf16)
        m_ref[...] = jnp.zeros(m_ref.shape, f32)
        l_ref[...] = jnp.ones(l_ref.shape, f32)
        acc_ref[...] = jnp.zeros(acc_ref.shape, f32)
        wait(cx)

        def xstep(r, carry):
            for k in range(NX):
                wait(xpiece(0, r, k) + xpiece(1, r, k))
                start(1, xpiece(1, r, k + ahead[1]))
                start(0, xpiece(0, r, k + ahead[0]))
            return carry

        npeel = -(-max(ahead) // NX)
        lax.fori_loop(0, NRS - npeel, xstep, 0)
        for r in range(NRS - npeel, NRS):
            xstep(r, 0)
        z = zref[...][0, 0]
        for b in range(2):
            xv = jnp.broadcast_to(xbuf[b, 0], (NU, D))
            for t in range(NB):
                xb[b, t] = xv[:, t * 128:(t + 1) * 128]
        for t in range(3):
            z = spin(z, SPIN1 if t == 0 else SPIN)
            start(1, piece(1, 0, 0, ahead[1] + t, z))
            start(0, piece(0, 0, 0, ahead[0] + t))

        def phase0(g, carry):
            segment(0, g, lambda: qproj(g))
            return carry

        lax.fori_loop(0, NG, phase0, 0)

        q0 = q_ref[0]
        s0 = segment(1, 0, lambda: qk(q0, 0, 0, None))
        s_ref[...] = lax.fori_loop(1, NU, lambda u, s: segment(1, u, lambda: qk(q0, 0, u, s)), s0)

        def main(a, carry):
            phase(a)
            return carry

        lax.fori_loop(2, NC - 1, main, 0)
        phase(NC - 1, hi=NU - (max(AHEAD) + 3) // 4)

        st = {}
        q = q_ref[NG - 1]

        def w0():
            st["p"], st["acc"] = softmax(None)
            st["s"] = None
            for u in range(0, 3):
                st["s"] = qk(q, NC - 1, u, st["s"])

        def w1():
            for u in range(3, 6):
                st["s"] = qk(q, NC - 1, u, st["s"])
            for u in range(0, 3):
                st["acc"] = pv(st["p"], NC - 2, u, st["acc"])

        def w2():
            for u in range(6, NU):
                st["s"] = qk(q, NC - 1, u, st["s"])
            for u in range(3, NU):
                st["acc"] = pv(st["p"], NC - 2, u, st["acc"])
            s_ref[...] = st["s"]
            acc_ref[...] = st["acc"]

        def w3():
            st["p"], st["acc"] = softmax(None)
            for v in (0, HG, 1, HG + 1):
                outproj(ocur_ref[...], NG - 2, v)

        def w4():
            for u in range(NU):
                st["acc"] = pv(st["p"], NC - 1, u, st["acc"])
            acc_ref[...] = st["acc"]

        def w5():
            o = normalized()
            st["o"] = o.astype(bf16)
            st["last"] = [jnp.broadcast_to(o[(b + 1) * HG - 1:(b + 1) * HG], (NU, DH)).astype(bf16)
                          for b in range(2)]
            for v in (2, HG + 2, 3, HG + 3):
                outproj(ocur_ref[...], NG - 2, v)

        def w6():
            for v in (0, HG, 1, HG + 1):
                outproj(st["o"], NG - 1, v)

        def w7():
            for v in (2, HG + 2):
                outproj(st["o"], NG - 1, v)
            out = out_ref[...]
            st["part"] = [jnp.sum(out[b * HG:(b + 1) * HG], axis=0, keepdims=True) for b in range(2)]

        def w8():
            for b in range(2):
                r = jnp.dot(st["last"][b], wor[b, (H - 1) * DH:H * DH, :], preferred_element_type=f32)
                o_ref[0, :, b * D:(b + 1) * D] = (st["part"][b] + r[0:1]).astype(o_ref.dtype)

        w0()
        for e, w in enumerate((w1, w2, w3, w4, w5, w6, w7, w8)):
            segment(NC, e, w)

    return pl.pallas_call(
        kernel,
        out_shape=jax.ShapeDtypeStruct((1, 1, 2 * D), bf16),
        in_specs=[pl.BlockSpec(memory_space=pl.ANY)] * 10,
        out_specs=pl.BlockSpec(memory_space=pltpu.VMEM),
        scratch_shapes=[
            pltpu.VMEM((2, 1, 1, D), bf16),
            pltpu.VMEM((2, NB, NU, 128), bf16),
            pltpu.VMEM((4, NU, R, DH), bf16),
            pltpu.VMEM((4, NU, R, DH), bf16),
            pltpu.VMEM((2, NG, NB, 128, GW), bf16),
            pltpu.VMEM((2, H * DH, D), bf16),
            pltpu.VMEM((8, 128), jnp.int32),
            pltpu.VMEM((NU, R), f32),
            pltpu.VMEM((NU, DH), f32),
            pltpu.VMEM((NU, DH), f32),
            pltpu.VMEM((NU, DH), f32),
            pltpu.VMEM((NG, NU, DH), bf16),
            pltpu.VMEM((NU, DH), bf16),
            pltpu.VMEM((NU, D), f32),
            pltpu.SemaphoreType.DMA((4,)),
        ],
        compiler_params=pltpu.CompilerParams(
            vmem_limit_bytes=64 * 1024 * 1024, disable_bounds_checks=True),
    )(A_x, A_k_cache, A_v_cache, A_wq.reshape(NB, 128, H * DH), A_wo,
      B_x, B_k_cache, B_v_cache, B_wq.reshape(NB, 128, H * DH), B_wo)
```

```python
import jax
import jax.numpy as jnp
from jax import lax
import jax.experimental.pallas as pl
import jax.experimental.pallas.tpu as pltpu

H, DH = 32, 128
HG = 4
NU = 2 * HG
R = 512
KR = 16
WR = 32
AHEAD = (20, 12)
SPIN0, SPIN1, SPIN = 50, 30, 54


@jax.jit
def pallas_concat_heads__sliding_block_cached__sliding_block_cached__decode_kernel(
    A_x: jax.Array,
    A_k_cache: jax.Array,
    A_v_cache: jax.Array,
    A_wq: jax.Array,
    A_wo: jax.Array,
    B_x: jax.Array,
    B_k_cache: jax.Array,
    B_v_cache: jax.Array,
    B_wq: jax.Array,
    B_wo: jax.Array,
):
    S = A_k_cache.shape[2]
    D = A_x.shape[2]
    W = min(4096, max(256, S // 4))
    scale = DH ** -0.5
    CPG = W // R
    NG = H // HG
    NC = NG * CPG
    NB = D // 128
    GW = HG * DH
    NRS = GW // WR
    assert A_x.shape == (1, 1, 512) and A_k_cache.shape == (1, H, S, DH)
    assert CPG == NU and NG == NU and R == 4 * KR * NU and NRS * 8 == 128
    f32, bf16 = jnp.float32, jnp.bfloat16

    def kernel(ax, ak, av, awq, awo, bx, bk, bv, bwq, bwo, o_ref,
               xbuf, xb, kbuf, vbuf, wqr, wor, zref,
               s_ref, m_ref, l_ref, acc_ref, q_ref, ocur_ref, ocol_ref, out_ref, sems):
        kv_hbm = ((ak, av), (bk, bv))
        wq_hbm = (awq, bwq)
        wo_hbm = (awo, bwo)
        kv_buf = (kbuf, vbuf)

        def static(v):
            return isinstance(v, int)

        def shr(v, n):
            return v >> n if static(v) else lax.shift_right_logical(v, n)

        def band(v, m):
            return v & m if static(v) else lax.bitwise_and(v, m)

        def mult(v, m):
            return v if static(v) else pl.multiple_of(v, m)

        def gmap(b, g):
            return g ^ b if static(g) else lax.bitwise_xor(g, b)

        def paced(v, z, hi):
            return v if z is None else jnp.clip(v + z, 0, hi)

        def spin(z, n):
            for _ in range(n):
                z = z * z
            return z

        def kv_piece(b, c, n, z=None):
            h0 = paced(gmap(b, shr(c, 3)) * HG, z, H - HG)
            row = mult(n * KR, KR)
            src_row = mult(S - W + band(c, CPG - 1) * R + row, KR)
            return [pltpu.make_async_copy(
                kv_hbm[b][kv].at[0, pl.ds(h0, HG), pl.ds(src_row, KR), :],
                kv_buf[kv].at[band(c, 3), pl.ds(b * HG, HG), pl.ds(row, KR), :],
                sems.at[band(c, 3)]) for kv in range(2)]

        def wq_piece(b, g, r, sem, z=None):
            return [pltpu.make_async_copy(
                wq_hbm[b].at[:, pl.ds(mult(paced(r, z, NRS - 1) * 8, 8), 8), pl.ds(g * GW, GW)],
                wqr.at[b, gmap(b, g), :, pl.ds(mult(r * 8, 8), 8), :], sem)]

        def wo_piece(b, g, r, sem, z=None):
            return [pltpu.make_async_copy(
                wo_hbm[b].at[pl.ds(mult(gmap(b, g) * GW + paced(r, z, NRS - 1) * WR, WR), WR), :],
                wor.at[b, pl.ds(mult(g * GW + r * WR, WR), WR), :], sem)]

        def piece(b, a, u, t, z=None):
            u, t = u + t // 4, t % 4
            a, u = a + shr(u, 3), band(u, 7)
            if not static(a) or a < NC:
                return kv_piece(b, a, 4 * u + t, z)
            if a > NC:
                return []
            r = 4 * (u & 3) + t if u >= 6 else 4 * ((u & 2) + (t & 1)) + 2 * (u & 1) + (t >> 1)
            return wo_piece(b, NG - 2 + (u >> 2), r, sems.at[(0, 0, 1, 1, 2, 2, 3, 0)[u]], z)

        def start(b, copies):
            for c in copies:
                c.start(priority=1 - b)

        def wait(copies):
            for c in copies:
                c.wait()

        def segment(a, u, work):
            for b in range(2):
                for t in range(4):
                    wait(piece(b, a, u, t))
            more = not (static(a) and static(u) and 32 * a + 4 * u + 1 + AHEAD[1] >= 32 * (NC + 1))
            z = zref[...][0, 0] if more else None
            start(1, piece(1, a, u, AHEAD[1]))
            start(0, piece(0, a, u, AHEAD[0]))
            res = work()
            for t in range(1, 4):
                if more:
                    z = spin(z, SPIN1 if t == 1 else SPIN)
                    start(1, piece(1, a, u, t + AHEAD[1], z))
                start(0, piece(0, a, u, t + AHEAD[0]))
            return res

        row_n = lax.broadcasted_iota(jnp.int32, (NU, DH), 0)
        row_w = lax.broadcasted_iota(jnp.int32, (NU, R), 0)

        def qk(q, c, u, s):
            r = lax.dot_general(q, kbuf[band(c, 3), u], (((1,), (1,)), ((), ())),
                                preferred_element_type=f32)
            return r if s is None else jnp.where(row_w == u, r, s)

        def pv(p, c, u, acc):
            r = jnp.dot(p, vbuf[band(c, 3), u], preferred_element_type=f32)
            return jnp.where(row_n == u, acc + r, acc)

        def softmax(first):
            s = s_ref[...]
            mx = jnp.broadcast_to(jnp.max(s, axis=-1, keepdims=True), (NU, DH))
            m_old = m_ref[...]
            m_new = jnp.maximum(m_old, mx)
            if first is not None:
                m_new = jnp.where(first, mx, m_new)
            ps = [jnp.exp((s[:, t * 128:(t + 1) * 128] - m_new) * scale) for t in range(R // 128)]
            alpha = jnp.exp((m_old - m_new) * scale)
            l_old = l_ref[...] * alpha
            acc = acc_ref[...] * alpha
            if first is not None:
                l_old = jnp.where(first, 0.0, l_old)
                acc = jnp.where(first, 0.0, acc)
            m_ref[...] = m_new
            l_ref[...] = l_old + ((ps[0] + ps[1]) + (ps[2] + ps[3]))
            return jnp.concatenate(ps, axis=1).astype(bf16), acc

        def normalized():
            return acc_ref[...] / jnp.sum(l_ref[...], axis=-1, keepdims=True)

        def qproj(g):
            q = jnp.zeros((NU, DH), f32)
            for b in range(2):
                r = jnp.dot(xb[b, 0], wqr[b, g, 0], preferred_element_type=f32)
                for t in range(1, NB):
                    r = r + jnp.dot(xb[b, t], wqr[b, g, t], preferred_element_type=f32)
                for hh in range(HG):
                    q = jnp.where(row_n == b * HG + hh, r[:, hh * DH:(hh + 1) * DH], q)
            q_ref[g] = q.astype(bf16)

        def outproj(o, g, v, valid=None):
            r0 = mult(g * GW + band(v, HG - 1) * DH, DH)
            r = jnp.dot(o, wor[shr(v, 2), pl.ds(r0, DH), :], preferred_element_type=f32)
            out = out_ref[...]
            sel = row_w == (v if valid is None else jnp.where(valid, v, -1))
            out_ref[...] = jnp.where(sel, out + r, out)

        def head_work(a):
            q = q_ref[shr(a - 1, 3)]
            v = band(a - 2, 7)
            first = v == 0
            o = jnp.where(first, normalized().astype(bf16), ocur_ref[...])
            ocur_ref[...] = o
            g1 = shr(a - 2, 3)
            outproj(o, jnp.clip(g1 - 1, 0, NG - 3), v, jnp.logical_and(g1 >= 1, g1 <= NG - 2))
            p, acc = softmax(first)
            return q, p, qk(q, a - 1, 0, None), pv(p, a - 2, 0, acc)

        def phase(a, hi=NU):
            q, p, s, acc = segment(a, 0, lambda: head_work(a))

            def body(u, carry):
                return segment(a, u, lambda: (qk(q, a - 1, u, carry[0]), pv(p, a - 2, u, carry[1])))

            carry = lax.fori_loop(1, hi, body, (s, acc))
            for u in range(hi, NU):
                carry = body(u, carry)
            s_ref[...] = carry[0]
            acc_ref[...] = carry[1]

        order = []
        for g in range(NG):
            order.append((wq_piece, g))
            if g % 4 != 3:
                order.append((wo_piece, g - g // 4))
        NX = len(order)
        ahead = [n - 3 for n in AHEAD]
        xsem = sems.at[3]

        def xpiece(b, r, k, z=None):
            r, k = r + k // NX, k % NX
            if static(r) and r >= NRS:
                return piece(b, 0, 0, (r - NRS) * NX + k, z)
            return order[k][0](b, order[k][1], r, xsem, z)

        cx = [pltpu.make_async_copy(ax, xbuf.at[0], xsem), pltpu.make_async_copy(bx, xbuf.at[1], xsem)]
        start(0, xpiece(0, 0, 0))
        start(1, xpiece(1, 0, 0))
        zref[...] = jnp.zeros(zref.shape, jnp.int32)
        for k in range(1, ahead[0]):
            start(0, xpiece(0, 0, k))
        start(0, cx)
        z = zref[...][0, 0]
        for k in range(1, ahead[1]):
            if k > 1:
                z = spin(z, SPIN0)
            start(1, xpiece(1, 0, k, z))
        out_ref[...] = jnp.zeros(out_ref.shape, f32)
        ocur_ref[...] = jnp.zeros(ocur_ref.shape, bf16)
        m_ref[...] = jnp.zeros(m_ref.shape, f32)
        l_ref[...] = jnp.ones(l_ref.shape, f32)
        acc_ref[...] = jnp.zeros(acc_ref.shape, f32)
        wait(cx)

        def xstep(r, carry):
            for k in range(NX):
                wait(xpiece(0, r, k) + xpiece(1, r, k))
                start(1, xpiece(1, r, k + ahead[1]))
                start(0, xpiece(0, r, k + ahead[0]))
            return carry

        npeel = -(-max(ahead) // NX)
        lax.fori_loop(0, NRS - npeel, xstep, 0)
        for r in range(NRS - npeel, NRS):
            xstep(r, 0)
        z = zref[...][0, 0]
        for b in range(2):
            xv = jnp.broadcast_to(xbuf[b, 0], (NU, D))
            for t in range(NB):
                xb[b, t] = xv[:, t * 128:(t + 1) * 128]
        for t in range(3):
            z = spin(z, SPIN1 if t == 0 else SPIN)
            start(1, piece(1, 0, 0, ahead[1] + t, z))
            start(0, piece(0, 0, 0, ahead[0] + t))

        def phase0(g, carry):
            segment(0, g, lambda: qproj(g))
            return carry

        lax.fori_loop(0, NG, phase0, 0)

        q0 = q_ref[0]
        s0 = segment(1, 0, lambda: qk(q0, 0, 0, None))
        s_ref[...] = lax.fori_loop(1, NU, lambda u, s: segment(1, u, lambda: qk(q0, 0, u, s)), s0)

        def main(a, carry):
            phase(a)
            return carry

        lax.fori_loop(2, NC - 1, main, 0)
        phase(NC - 1, hi=NU - (max(AHEAD) + 3) // 4)

        st = {}
        q = q_ref[NG - 1]

        def w0():
            st["p"], st["acc"] = softmax(None)
            st["s"] = None
            for u in range(0, 3):
                st["s"] = qk(q, NC - 1, u, st["s"])

        def w1():
            for u in range(3, 6):
                st["s"] = qk(q, NC - 1, u, st["s"])
            for u in range(0, 3):
                st["acc"] = pv(st["p"], NC - 2, u, st["acc"])

        def w2():
            for u in range(6, NU):
                st["s"] = qk(q, NC - 1, u, st["s"])
            for u in range(3, NU):
                st["acc"] = pv(st["p"], NC - 2, u, st["acc"])
            s_ref[...] = st["s"]
            acc_ref[...] = st["acc"]

        def w3():
            st["p"], st["acc"] = softmax(None)
            for v in (0, HG, 1, HG + 1):
                outproj(ocur_ref[...], NG - 2, v)

        def w4():
            for u in range(NU):
                st["acc"] = pv(st["p"], NC - 1, u, st["acc"])
            acc_ref[...] = st["acc"]

        def w5():
            st["o"] = normalized().astype(bf16)
            o = st["o"].astype(f32)
            for b in range(2):
                ocol_ref[b] = jnp.broadcast_to(o[(b + 1) * HG - 1:(b + 1) * HG], (DH, DH)).T
            for v in (2, HG + 2, 3, HG + 3):
                outproj(ocur_ref[...], NG - 2, v)

        def w6():
            for v in (0, HG, 1, HG + 1):
                outproj(st["o"], NG - 1, v)

        def w7():
            for v in (2, HG + 2):
                outproj(st["o"], NG - 1, v)
            out = out_ref[...]
            st["part"] = [jnp.where(shr(row_w, 2) == b, out, 0.0) for b in range(2)]

        def w8():
            for b in range(2):
                w = wor[b, (H - 1) * DH:H * DH, :].astype(f32)
                prod = w * jnp.concatenate([ocol_ref[b]] * (D // DH), axis=1)
                terms = [prod[i:i + NU] for i in range(0, DH, NU)]
                while len(terms) > 1:
                    terms = [terms[i] + terms[i + 1] for i in range(0, len(terms), 2)]
                res = jnp.sum(st["part"][b] + terms[0], axis=0, keepdims=True)
                o_ref[0, :, b * D:(b + 1) * D] = res.astype(o_ref.dtype)

        w0()
        for e, w in enumerate((w1, w2, w3, w4, w5, w6, w7, w8)):
            segment(NC, e, w)

    return pl.pallas_call(
        kernel,
        out_shape=jax.ShapeDtypeStruct((1, 1, 2 * D), bf16),
        in_specs=[pl.BlockSpec(memory_space=pl.ANY)] * 10,
        out_specs=pl.BlockSpec(memory_space=pltpu.VMEM),
        scratch_shapes=[
            pltpu.VMEM((2, 1, 1, D), bf16),
            pltpu.VMEM((2, NB, NU, 128), bf16),
            pltpu.VMEM((4, NU, R, DH), bf16),
            pltpu.VMEM((4, NU, R, DH), bf16),
            pltpu.VMEM((2, NG, NB, 128, GW), bf16),
            pltpu.VMEM((2, H * DH, D), bf16),
            pltpu.VMEM((8, 128), jnp.int32),
            pltpu.VMEM((NU, R), f32),
            pltpu.VMEM((NU, DH), f32),
            pltpu.VMEM((NU, DH), f32),
            pltpu.VMEM((NU, DH), f32),
            pltpu.VMEM((NG, NU, DH), bf16),
            pltpu.VMEM((NU, DH), bf16),
            pltpu.VMEM((2, DH, DH), f32),
            pltpu.VMEM((NU, D), f32),
            pltpu.SemaphoreType.DMA((4,)),
        ],
        compiler_params=pltpu.CompilerParams(
            vmem_limit_bytes=64 * 1024 * 1024, disable_bounds_checks=True),
    )(A_x, A_k_cache, A_v_cache, A_wq.reshape(NB, 128, H * DH), A_wo,
      B_x, B_k_cache, B_v_cache, B_wq.reshape(NB, 128, H * DH), B_wo)
```
